```python
import jax
import jax.numpy as jnp

def _softmax(x, axis=-1):
    return jax.nn.softmax(x, axis=axis)
def _gelu(x):
    return jax.nn.gelu(x, approximate=True)
def _silu(x):
    return jax.nn.silu(x)
def _sigmoid(x):
    return jax.nn.sigmoid(x)
def _layernorm(x, axis=-1, eps=1e-5):
    m = jnp.mean(x, axis=axis, keepdims=True)
    v = jnp.var(x, axis=axis, keepdims=True)
    return (x - m) / jnp.sqrt(v + eps)
def _scatter_add(tgt, idx, src, axis=0):
    return tgt.at[idx].add(src)
def _segment_sum(src, seg, n):
    return jax.ops.segment_sum(src, seg, n)
class _Rng:
    def __init__(self, key):
        self._k = key
    def _next(self):
        self._k, sub = jax.random.split(self._k)
        return sub
    def normal(self, shape):
        return jax.random.normal(self._next(), shape, dtype=jnp.bfloat16)
    def randint(self, lo, hi, shape):
        return jax.random.randint(self._next(), shape, lo, hi, dtype=jnp.int32)
    def uniform(self, shape, lo=0.0, hi=1.0):
        return jax.random.uniform(self._next(), shape, jnp.bfloat16, lo, hi)
    def permutation(self, n):
        return jax.random.permutation(self._next(), n)


kernel_name = 'recurrent_scan__compressed_kv_cla__moe_arch_mod__decode'

def setup_inputs():
    _rng = _Rng(jax.random.key(int.from_bytes(__import__("os").urandom(4), "little")))
    _w = (lambda a: (lambda t: t.astype(jnp.bfloat16) if jnp.issubdtype(t.dtype, jnp.floating) else t)(jnp.asarray(a)))
    def _A_setup():
        B, H, Sq, Sk, D, M = 4, 32, 1, 4096, 128, 576
        Dc = 4 * D
        return {
            "x": _w((lambda *s: _rng.normal(s) * 0.05)(B, Sq, M)),
            "c_kv": _w((lambda *s: _rng.normal(s) * 0.05)(B, Sk, Dc)),
            "w_q": _w((lambda *s: _rng.normal(s) * 0.05)(M, H, D) * (M ** -0.5)),
            "w_uk": _w((lambda *s: _rng.normal(s) * 0.05)(Dc, H, D) * (Dc ** -0.5)),
            "w_uv": _w((lambda *s: _rng.normal(s) * 0.05)(Dc, H, D) * (Dc ** -0.5)),
            "w_o": _w((lambda *s: _rng.normal(s) * 0.05)(H, D, M) * ((H * D) ** -0.5)),
        }
    _A_in = _A_setup()

    def _B_setup():
        B, S, D, F, C = 4, 1, 576, 4608, 1
        return {
            "x": _w((lambda *s: _rng.normal(s) * 0.05)(B, S, D)),
            "w_r": _w((lambda *s: _rng.normal(s) * 0.05)(D)),
            "w_gate": _w((lambda *s: _rng.normal(s) * 0.05)(D, F)),
            "w_up": _w((lambda *s: _rng.normal(s) * 0.05)(D, F)),
            "w_down": _w((lambda *s: _rng.normal(s) * 0.05)(F, D)),
        }
    _B_in = _B_setup()

    return {
        "A_x": _A_in["x"],
        "A_c_kv": _A_in["c_kv"],
        "A_w_q": _A_in["w_q"],
        "A_w_uk": _A_in["w_uk"],
        "A_w_uv": _A_in["w_uv"],
        "A_w_o": _A_in["w_o"],
        "B_x": _B_in["x"],
        "B_w_r": _B_in["w_r"],
        "B_w_gate": _B_in["w_gate"],
        "B_w_up": _B_in["w_up"],
        "B_w_down": _B_in["w_down"],
    }

def reference(A_x, A_c_kv, A_w_q, A_w_uk, A_w_uv, A_w_o, B_x, B_w_r, B_w_gate, B_w_up, B_w_down):
    def _A_ref(x, c_kv, w_q, w_uk, w_uv, w_o):
        B, Sq, M = x.shape[0], x.shape[1], x.shape[2]
        Sk = c_kv.shape[1]
        H, D = w_q.shape[1], w_q.shape[2]
        q = jnp.einsum("bqm,mhd->bhqd", x, w_q)
        k = jnp.einsum("bkc,chd->bhkd", c_kv, w_uk)
        v = jnp.einsum("bkc,chd->bhkd", c_kv, w_uv)
        scores = jnp.einsum("bhqd,bhkd->bhqk", q, k) * (D ** -0.5)
        off = Sk - Sq
        qi = jnp.arange(Sq)[:, None]
        kj = jnp.arange(Sk)[None, :]
        cmask = kj <= (qi + off)
        scores = jnp.where(cmask[None, None], scores, -1e9)
        p = _softmax(scores, axis=-1)
        ctx = jnp.einsum("bhqk,bhkd->bhqd", p, v)
        return jnp.einsum("bhqd,hdm->bqm", ctx, w_o)

    def _B_ref(x, w_r, w_gate, w_up, w_down):
        B, S, D = x.shape
        C = 1
        r = x @ w_r
        idx = jnp.argsort(-r, axis=-1)[:, :C]
        idx_e = jnp.repeat(idx.reshape(B, C, 1), D, axis=2)
        x_sel = jnp.take_along_axis(x, idx_e, axis=1)
        g = _silu(x_sel @ w_gate)
        u = x_sel @ w_up
        y = (g * u) @ w_down
        r_sel = _sigmoid(jnp.take_along_axis(r, idx, axis=1))
        y = y * r_sel.reshape(B, C, 1)
        b_off = (jnp.arange(B) * S).reshape(B, 1)
        flat_idx = (idx + b_off).reshape(B * C)
        zero = (x * 0.0).reshape(B * S, D)
        upd = _scatter_add(zero, flat_idx, y.reshape(B * C, D), axis=0)
        return x + upd.reshape(B, S, D)

    x = A_x
    xn = _layernorm(x, axis=-1)
    s = _A_ref(xn, A_c_kv, A_w_q, A_w_uk, A_w_uv, A_w_o)
    g = _silu(_B_ref(xn, B_w_r, B_w_gate, B_w_up, B_w_down))
    return x + s * g
```

```python
import jax
import jax.numpy as jnp
from jax import lax
from jax.experimental import pallas as pl
from jax.experimental.pallas import tpu as pltpu

B, H, SK, D, M, DC, F = 4, 32, 4096, 128, 576, 512, 4608
KC = 1024
NC = 512
WO_CHUNKS = (6, 4, 3, 1, 1, 1)
f32 = jnp.float32
bf16 = jnp.bfloat16
u32 = jnp.uint32


def _dot(a, b):
    return jnp.dot(a, b, preferred_element_type=f32)


def _dot_nt(a, b):
    return lax.dot_general(a, b, (((1,), (1,)), ((), ())), preferred_element_type=f32)


def _iota(shape, dim):
    return lax.broadcasted_iota(jnp.int32, shape, dim)


def _kernel(x_hbm, wr_hbm, wq_hbm, wuk_hbm, ckv_hbm, wuv_hbm, wo_hbm, wg_hbm, wu_hbm, wd_hbm,
            o_ref,
            x_v, wr_v, wq_v, wuk_v, ckv_v, wuv_v, wo_v, wg_v, wu_v, wd_v,
            q_s, qa_s, s_s, cc_s, lc_s, ctx_s, h_s, sems):
    cps = {}

    def add(name, src, dst):
        cps[name] = pltpu.make_async_copy(src, dst, sems.at[len(cps)])

    add('x', x_hbm, x_v)
    add('wr', wr_hbm, wr_v)
    add('wq', wq_hbm.bitcast(u32), wq_v)
    add('wuk', wuk_hbm.bitcast(u32), wuk_v)
    for b in range(B):
        add(f'ckv{b}', ckv_hbm.at[b], ckv_v.at[b])
    add('wuv', wuv_hbm.bitcast(u32), wuv_v)
    add('wg', wg_hbm, wg_v)
    add('wu', wu_hbm, wu_v)
    add('wd', wd_hbm, wd_v)
    j0 = 0
    for ci, nj in enumerate(WO_CHUNKS):
        rows = pl.ds(j0 * 2 * M, nj * 2 * M)
        add(f'wo{ci}', wo_hbm.at[rows], wo_v.at[rows])
        j0 += nj
    for c in cps.values():
        c.start()

    cps['x'].wait()
    cps['wr'].wait()
    x = x_v[...].astype(f32)
    mu = jnp.mean(x, axis=-1, keepdims=True)
    xc = x - mu
    var = jnp.mean(xc * xc, axis=-1, keepdims=True)
    xn = (xc / jnp.sqrt(var + 1e-5)).astype(bf16).astype(f32)
    wr = wr_v[...].astype(f32).reshape(1, M)
    r = jnp.sum(xn * wr, axis=-1, keepdims=True)
    xn8 = jnp.concatenate([xn, xn], axis=0).astype(bf16)
    E = (_iota((128, 256), 1) // 2 == _iota((128, 256), 0)).astype(f32).astype(bf16)
    ET = (_iota((256, 128), 0) // 2 == _iota((256, 128), 1)).astype(f32).astype(bf16)
    parts = [_dot(xn8[:, 128 * k:128 * (k + 1)], E) for k in range(4)]
    parts.append(_dot(xn8[:, 512:576], E[:64, :128]))
    lx = jnp.concatenate(parts, axis=1)
    lx = jnp.where(_iota((8, 2 * M), 0) // 4 == _iota((8, 2 * M), 1) % 2, lx, 0.0).astype(bf16)

    cps['wq'].wait()

    def body_q(jj, _):
        ws = [pltpu.bitcast(wq_v[pl.ds(4 * jj + i, M, stride=16), :], bf16) for i in range(4)]
        res = _dot(lx, jnp.concatenate(ws, axis=1)) * (D ** -0.5)
        for i in range(4):
            q_s[pl.ds(pl.multiple_of(8 * (4 * jj + i), 8), 8), :] = res[:, 128 * i:128 * (i + 1)]
        return 0
    lax.fori_loop(0, 4, body_q, 0)

    cps['wuk'].wait()
    pm = _iota((8, 2 * DC), 0) // 4 == _iota((8, 2 * DC), 1) % 2

    def body_qa(j, _):
        w = pltpu.bitcast(wuk_v[pl.ds(j, DC, stride=16), :], bf16)
        rows = pl.ds(pl.multiple_of(8 * j, 8), 8)
        lc_s[rows, :] = jnp.where(pm, _dot_nt(q_s[rows, :].astype(bf16), w), 0.0)
        return 0
    lax.fori_loop(0, 16, body_qa, 0)
    rall = lc_s[...].astype(bf16)
    for k in range(4):
        qa_s[k] = _dot(rall[:, 256 * k:256 * (k + 1)], ET)

    for b in range(B):
        cps[f'ckv{b}'].wait()
        qa = jnp.concatenate([qa_s[k, pl.ds(b, H, stride=4), :] for k in range(4)], axis=1).astype(bf16)

        def body_s(i, mx, b=b, qa=qa):
            s = _dot_nt(qa, ckv_v[b, pl.ds(pl.multiple_of(i * KC, KC), KC), :])
            s_s[i] = s
            for t in range(KC // 128):
                mx = jnp.maximum(mx, s[:, 128 * t:128 * (t + 1)])
            return mx
        mx = lax.fori_loop(0, SK // KC, body_s, jnp.full((H, 128), -jnp.inf, f32))
        mx = jnp.max(mx, axis=1, keepdims=True)

        def body_pv(i, carry, b=b, mx=mx):
            acc, l = carry
            p = jnp.exp(s_s[i] - mx)
            for t in range(KC // 128):
                l = l + p[:, 128 * t:128 * (t + 1)]
            kk = ckv_v[b, pl.ds(pl.multiple_of(i * KC, KC), KC), :]
            return acc + _dot(p.astype(bf16), kk), l
        acc, l = lax.fori_loop(0, SK // KC, body_pv,
                               (jnp.zeros((H, DC), f32), jnp.zeros((H, 128), f32)))
        acc = acc / jnp.sum(l, axis=1, keepdims=True)
        for k in range(4):
            cc_s[k, pl.ds(b, H, stride=4), :] = acc[:, 128 * k:128 * (k + 1)]

    cps['wuv'].wait()
    pm2 = (_iota((128, 256), 0) // 4) % 2 == _iota((128, 256), 1) % 2
    for k in range(4):
        lc_s[:, 256 * k:256 * (k + 1)] = jnp.where(pm2, _dot(cc_s[k].astype(bf16), E), 0.0)

    def body_ctx(j, _):
        w = pltpu.bitcast(wuv_v[pl.ds(j, DC, stride=16), :], bf16)
        rows = pl.ds(pl.multiple_of(8 * j, 8), 8)
        ctx_s[rows, :] = _dot(lc_s[rows, :].astype(bf16), w)
        return 0
    lax.fori_loop(0, 16, body_ctx, 0)

    cps['wg'].wait()

    def body_g(i, _):
        cols = pl.ds(pl.multiple_of(i * NC, NC), NC)
        h_s[:, cols] = _dot(xn8, wg_v[:, cols])
        return 0
    lax.fori_loop(0, F // NC, body_g, 0)
    cps['wu'].wait()

    def body_u(i, _):
        cols = pl.ds(pl.multiple_of(i * NC, NC), NC)
        g = h_s[:, cols]
        h_s[:, cols] = g * jax.nn.sigmoid(g) * _dot(xn8, wu_v[:, cols])
        return 0
    lax.fori_loop(0, F // NC, body_u, 0)
    cps['wd'].wait()

    def body_d(i, y):
        cols = pl.ds(pl.multiple_of(i * NC, NC), NC)
        return y + _dot_nt(h_s[:, cols].astype(bf16), wd_v[:, cols])
    y = lax.fori_loop(0, F // NC, body_d, jnp.zeros((8, M), f32))
    t = xn + y[:4] * jax.nn.sigmoid(r)
    gate = t * jax.nn.sigmoid(t)

    def body_o(j, carry):
        a0, a1 = carry
        cj = ctx_s[pl.ds(pl.multiple_of(8 * j, 8), 8), :].astype(bf16)
        w0 = wo_v[pl.ds(pl.multiple_of(2 * j * M, 64), M), :]
        w1 = wo_v[pl.ds(pl.multiple_of((2 * j + 1) * M, 64), M), :]
        return a0 + _dot_nt(cj, w0), a1 + _dot_nt(cj, w1)
    carry = (jnp.zeros((8, M), f32), jnp.zeros((8, M), f32))
    j0 = 0
    for ci, nj in enumerate(WO_CHUNKS):
        cps[f'wo{ci}'].wait()
        carry = body_o(j0, carry) if nj == 1 else lax.fori_loop(j0, j0 + nj, body_o, carry)
        j0 += nj
    a0, a1 = carry
    o_ref[...] = (x + (a0[:4] + a1[4:]) * gate).astype(o_ref.dtype)


@jax.jit
def pallas_recurrent_scan__compressed_kv_cla__moe_arch_mod__decode_kernel(
    A_x: jax.Array,
    A_c_kv: jax.Array,
    A_w_q: jax.Array,
    A_w_uk: jax.Array,
    A_w_uv: jax.Array,
    A_w_o: jax.Array,
    B_x: jax.Array,
    B_w_r: jax.Array,
    B_w_gate: jax.Array,
    B_w_up: jax.Array,
    B_w_down: jax.Array,
):
    del B_x
    x = A_x.reshape(B, M)
    wq = A_w_q.reshape(M * H, D)
    wuk = A_w_uk.reshape(DC * H, D)
    wuv = A_w_uv.reshape(DC * H, D)
    wo = jnp.transpose(A_w_o, (0, 2, 1)).reshape(H * M, D)
    wd = B_w_down.T
    out = pl.pallas_call(
        _kernel,
        out_shape=jax.ShapeDtypeStruct((B, M), bf16),
        in_specs=[pl.BlockSpec(memory_space=pl.ANY)] * 10,
        out_specs=pl.BlockSpec(memory_space=pltpu.VMEM),
        scratch_shapes=[
            pltpu.VMEM((B, M), bf16),
            pltpu.VMEM((M,), bf16),
            pltpu.VMEM((M * H // 2, D), u32),
            pltpu.VMEM((DC * H // 2, D), u32),
            pltpu.VMEM((B, SK, DC), bf16),
            pltpu.VMEM((DC * H // 2, D), u32),
            pltpu.VMEM((H * M, D), bf16),
            pltpu.VMEM((M, F), bf16),
            pltpu.VMEM((M, F), bf16),
            pltpu.VMEM((M, F), bf16),
            pltpu.VMEM((128, 128), f32),
            pltpu.VMEM((4, 128, 128), f32),
            pltpu.VMEM((SK // KC, H, KC), f32),
            pltpu.VMEM((4, 128, 128), f32),
            pltpu.VMEM((128, 2 * DC), f32),
            pltpu.VMEM((128, 128), f32),
            pltpu.VMEM((8, F), f32),
            pltpu.SemaphoreType.DMA((12 + len(WO_CHUNKS),)),
        ],
        compiler_params=pltpu.CompilerParams(
            vmem_limit_bytes=100 * 1024 * 1024,
            disable_semaphore_checks=True,
        ),
    )(x, B_w_r, wq, wuk, A_c_kv, wuv, wo, B_w_gate, B_w_up, wd)
    return out.reshape(B, 1, M)
```

```python
import jax
import jax.numpy as jnp
from jax import lax
from jax.experimental import pallas as pl
from jax.experimental.pallas import tpu as pltpu

B, H, SK, D, M, DC, F = 4, 32, 4096, 128, 576, 512, 4608
KC = 1024
NC = 512
HR = M // 2
BOUNCE = (960, 960, 960)
EARLY = 3
WO_CHUNKS = (4, 3, 2, 1)
WD_CHUNKS = 3
UNROLL_O = 4
NBJ = sum(BOUNCE) // (2 * HR)
assert NBJ * 2 * HR == sum(BOUNCE) and NBJ + sum(WO_CHUNKS) + 1 == H // 2
assert EARLY * 2 * HR <= BOUNCE[0] + BOUNCE[1]
N_SEMS = 11 + WD_CHUNKS + len(WO_CHUNKS) + 2 + 2 * len(BOUNCE)
f32 = jnp.float32
bf16 = jnp.bfloat16
u32 = jnp.uint32


def _dot(a, b):
    return jnp.dot(a, b, preferred_element_type=f32)


def _dot_nt(a, b):
    return lax.dot_general(a, b, (((1,), (1,)), ((), ())), preferred_element_type=f32)


def _iota(shape, dim):
    return lax.broadcasted_iota(jnp.int32, shape, dim)


def _kernel(x_hbm, wr_hbm, wq_hbm, wuk_hbm, ckv_hbm, wuv_hbm, wo_hbm, wg_hbm, wu_hbm, wd_hbm,
            o_ref,
            x_v, wr_v, wq_v, wuk_v, ckv_v, wuv_v, wo_v, wg_v, wu_v, wd_v,
            q_s, qa_s, s_s, cc_s, lc_s, ctx_s, h_s, bounce_sm, sems):
    n_sem = [0]

    def copy(src, dst):
        c = pltpu.make_async_copy(src, dst, sems.at[n_sem[0]])
        n_sem[0] += 1
        return c

    wo32 = wo_hbm.bitcast(u32)

    def wo_copy(row0, nrows):
        return copy(wo32.at[pl.ds(row0, nrows)], wo_v.at[pl.ds(row0, nrows)])

    c_x = copy(x_hbm, x_v)
    c_wr = copy(wr_hbm, wr_v)
    c_wq = copy(wq_hbm.bitcast(u32), wq_v)
    c_wuk = copy(wuk_hbm.bitcast(u32), wuk_v)
    c_ckv = [copy(ckv_hbm.at[b], ckv_v.at[b]) for b in range(B)]
    c_wuv = copy(wuv_hbm.bitcast(u32), wuv_v)
    c_wg = copy(wg_hbm, wg_v)
    c_wu = copy(wu_hbm, wu_v)
    fc = F // WD_CHUNKS
    c_wd = [copy(wd_hbm.at[:, pl.ds(i * fc, fc)], wd_v.at[:, pl.ds(i * fc, fc)])
            for i in range(WD_CHUNKS)]
    c_wo, j0 = [], NBJ
    for nj in WO_CHUNKS:
        c_wo.append(wo_copy(j0 * 2 * HR, nj * 2 * HR))
        j0 += nj
    c_wo_a = wo_copy((H - 2) * HR, HR)
    c_wo_b = wo_copy((H - 1) * HR, HR)
    b_in, b_out, r0 = [], [], 0
    for i, n in enumerate(BOUNCE):
        slot = bounce_sm.at[i % 2, pl.ds(0, n)]
        b_in.append(copy(wo32.at[pl.ds(r0, n)], slot))
        b_out.append(copy(slot, wo_v.at[pl.ds(r0, n)]))
        r0 += n
    assert n_sem[0] == N_SEMS

    for c in [c_x, c_wr, c_wq, b_in[0], b_in[1], c_wuk, *c_ckv, c_wuv, c_wg, c_wu,
              *c_wd, *c_wo, c_wo_a, c_wo_b]:
        c.start()

    cc_s[...] = jnp.zeros(cc_s.shape, f32)
    c_x.wait()
    c_wr.wait()
    x = x_v[...].astype(f32)
    mu = jnp.mean(x, axis=-1, keepdims=True)
    xc = x - mu
    var = jnp.mean(xc * xc, axis=-1, keepdims=True)
    xn = (xc / jnp.sqrt(var + 1e-5)).astype(bf16).astype(f32)
    wr = wr_v[...].astype(f32).reshape(1, M)
    r = jnp.sum(xn * wr, axis=-1, keepdims=True)
    xn8 = jnp.concatenate([xn, xn], axis=0).astype(bf16)
    E = (_iota((128, 256), 1) // 2 == _iota((128, 256), 0)).astype(f32).astype(bf16)
    ET = (_iota((256, 128), 0) // 2 == _iota((256, 128), 1)).astype(f32).astype(bf16)
    parts = [_dot(xn8[:, 128 * k:128 * (k + 1)], E) for k in range(4)]
    parts.append(_dot(xn8[:, 512:576], E[:64, :128]))
    lx = jnp.concatenate(parts, axis=1)
    lx = jnp.where(_iota((8, 2 * M), 0) // 4 == _iota((8, 2 * M), 1) % 2, lx, 0.0).astype(bf16)

    c_wq.wait()

    def body_q(jj, _):
        ws = [pltpu.bitcast(wq_v[pl.ds(4 * jj + i, M, stride=16), :], bf16) for i in range(4)]
        res = _dot(lx, jnp.concatenate(ws, axis=1)) * (D ** -0.5)
        for i in range(4):
            q_s[pl.ds(pl.multiple_of(8 * (4 * jj + i), 8), 8), :] = res[:, 128 * i:128 * (i + 1)]
        return 0
    lax.fori_loop(0, 4, body_q, 0)
    b_in[0].wait()
    b_out[0].start()

    c_wuk.wait()
    pm = _iota((8, 2 * DC), 0) // 4 == _iota((8, 2 * DC), 1) % 2

    def body_qa(j, _):
        w = pltpu.bitcast(wuk_v[pl.ds(j, DC, stride=16), :], bf16)
        rows = pl.ds(pl.multiple_of(8 * j, 8), 8)
        lc_s[rows, :] = jnp.where(pm, _dot_nt(q_s[rows, :].astype(bf16), w), 0.0)
        return 0
    lax.fori_loop(0, H // 2, body_qa, 0)
    rall = lc_s[...].astype(bf16)
    for k in range(4):
        qa_s[k] = _dot(rall[:, 256 * k:256 * (k + 1)], ET)

    for b in range(B):
        c_ckv[b].wait()
        if b == 2:
            b_in[1].wait()
            b_out[1].start()
            b_out[0].wait()
            b_in[2].start()
        qa = jnp.concatenate([qa_s[k, pl.ds(b, H, stride=4), :] for k in range(4)],
                             axis=1).astype(bf16)

        def body_s(i, mx, b=b, qa=qa):
            s = _dot_nt(qa, ckv_v[b, pl.ds(pl.multiple_of(i * KC, KC), KC), :])
            s_s[i] = s
            for t in range(KC // 128):
                mx = jnp.maximum(mx, s[:, 128 * t:128 * (t + 1)])
            return mx
        mx = lax.fori_loop(0, SK // KC, body_s, jnp.full((H, 128), -jnp.inf, f32))
        mx = jnp.max(mx, axis=1, keepdims=True)

        def body_pv(i, carry, b=b, mx=mx):
            acc, l = carry
            p = jnp.exp(s_s[i] - mx)
            for t in range(KC // 128):
                l = l + p[:, 128 * t:128 * (t + 1)]
            kk = ckv_v[b, pl.ds(pl.multiple_of(i * KC, KC), KC), :]
            return acc + _dot(p.astype(bf16), kk), l
        acc, l = lax.fori_loop(0, SK // KC, body_pv,
                               (jnp.zeros((H, DC), f32), jnp.zeros((H, 128), f32)))
        acc = acc / jnp.sum(l, axis=1, keepdims=True)
        for k in range(4):
            cc_s[k, pl.ds(b, H, stride=4), :] = acc[:, 128 * k:128 * (k + 1)]

    c_wuv.wait()
    pm2 = (_iota((128, 256), 0) // 4) % 2 == _iota((128, 256), 1) % 2
    for k in range(4):
        lc_s[:, 256 * k:256 * (k + 1)] = jnp.where(pm2, _dot(cc_s[k].astype(bf16), E), 0.0)

    def body_ctx(j, _):
        w = pltpu.bitcast(wuv_v[pl.ds(j, DC, stride=16), :], bf16)
        rows = pl.ds(pl.multiple_of(8 * j, 8), 8)
        ctx_s[rows, :] = _dot(lc_s[rows, :].astype(bf16), w)
        return 0
    lax.fori_loop(0, H // 2, body_ctx, 0)

    c_wg.wait()

    def body_g(i, _):
        cols = pl.ds(pl.multiple_of(i * NC, NC), NC)
        h_s[:, cols] = _dot(xn8, wg_v[:, cols])
        return 0
    lax.fori_loop(0, F // NC, body_g, 0)
    b_in[2].wait()
    b_out[2].start()
    c_wu.wait()

    def body_u(i, _):
        cols = pl.ds(pl.multiple_of(i * NC, NC), NC)
        g = h_s[:, cols]
        h_s[:, cols] = g * jax.nn.sigmoid(g) * _dot(xn8, wu_v[:, cols])
        return 0
    lax.fori_loop(0, F // NC, body_u, 0)

    def o_range(j0, nj, acc):
        assert nj <= UNROLL_O
        for j in range(j0, j0 + nj):
            cj = ctx_s[pl.ds(8 * j, 8), :].astype(bf16)
            w = pltpu.bitcast(wo_v[pl.ds(2 * j * HR, 2 * HR), :], bf16)
            acc = acc + _dot_nt(cj, w)
        return acc

    b_out[1].wait()
    acc = o_range(0, EARLY, jnp.zeros((8, 2 * M), f32))

    def body_d(i, y):
        cols = pl.ds(pl.multiple_of(i * NC, NC), NC)
        return y + _dot_nt(h_s[:, cols].astype(bf16), wd_v[:, cols])
    y = jnp.zeros((8, M), f32)
    for i in range(WD_CHUNKS):
        if i == WD_CHUNKS - 1:
            b_out[2].wait()
            acc = o_range(EARLY, NBJ - EARLY, acc)
        c_wd[i].wait()
        y = lax.fori_loop(i * (fc // NC), (i + 1) * (fc // NC), body_d, y)
    t = xn + y[:4] * jax.nn.sigmoid(r)
    gate = t * jax.nn.sigmoid(t)

    j0 = NBJ
    for c, nj in zip(c_wo, WO_CHUNKS):
        c.wait()
        acc = o_range(j0, nj, acc)
        j0 += nj
    c_wo_a.wait()
    cj = ctx_s[pl.ds(4 * (H - 2), 8), :]
    cl = jnp.concatenate([cj[4:], cj[:4]], axis=0).astype(bf16)
    w = pltpu.bitcast(wo_v[pl.ds((H - 2) * HR, HR), :], bf16)
    s = acc[:4, :M] + acc[4:, M:] + _dot_nt(cj.astype(bf16), w)[:4]
    base = x + s * gate
    c_wo_b.wait()
    w = pltpu.bitcast(wo_v[pl.ds((H - 1) * HR, HR), :], bf16)
    o_ref[...] = (base + _dot_nt(cl, w)[:4] * gate).astype(o_ref.dtype)


@jax.jit
def pallas_recurrent_scan__compressed_kv_cla__moe_arch_mod__decode_kernel(
    A_x: jax.Array,
    A_c_kv: jax.Array,
    A_w_q: jax.Array,
    A_w_uk: jax.Array,
    A_w_uv: jax.Array,
    A_w_o: jax.Array,
    B_x: jax.Array,
    B_w_r: jax.Array,
    B_w_gate: jax.Array,
    B_w_up: jax.Array,
    B_w_down: jax.Array,
):
    del B_x
    x = A_x.reshape(B, M)
    wq = A_w_q.reshape(M * H, D)
    wuk = A_w_uk.reshape(DC * H, D)
    wuv = A_w_uv.reshape(DC * H, D)
    wo = jnp.transpose(A_w_o, (0, 2, 1)).reshape(H * M, D)
    wd = B_w_down.T
    out = pl.pallas_call(
        _kernel,
        out_shape=jax.ShapeDtypeStruct((B, M), bf16),
        in_specs=[pl.BlockSpec(memory_space=pl.ANY)] * 10,
        out_specs=pl.BlockSpec(memory_space=pltpu.VMEM),
        scratch_shapes=[
            pltpu.VMEM((B, M), bf16),
            pltpu.VMEM((M,), bf16),
            pltpu.VMEM((M * H // 2, D), u32),
            pltpu.VMEM((DC * H // 2, D), u32),
            pltpu.VMEM((B, SK, DC), bf16),
            pltpu.VMEM((DC * H // 2, D), u32),
            pltpu.VMEM((H * HR, D), u32),
            pltpu.VMEM((M, F), bf16),
            pltpu.VMEM((M, F), bf16),
            pltpu.VMEM((M, F), bf16),
            pltpu.VMEM((128, 128), f32),
            pltpu.VMEM((4, 128, 128), f32),
            pltpu.VMEM((SK // KC, H, KC), f32),
            pltpu.VMEM((4, 128, 128), f32),
            pltpu.VMEM((128, 2 * DC), f32),
            pltpu.VMEM((128, 128), f32),
            pltpu.VMEM((8, F), f32),
            pltpu.SMEM((2, max(BOUNCE), D), u32),
            pltpu.SemaphoreType.DMA((N_SEMS,)),
        ],
        compiler_params=pltpu.CompilerParams(
            vmem_limit_bytes=100 * 1024 * 1024,
            disable_semaphore_checks=True,
        ),
    )(x, B_w_r, wq, wuk, A_c_kv, wuv, wo, B_w_gate, B_w_up, wd)
    return out.reshape(B, 1, M)
```

```python
import jax
import jax.numpy as jnp
from jax import lax
from jax.experimental import pallas as pl
from jax.experimental.pallas import tpu as pltpu

B, H, SK, D, M, DC, F = 4, 32, 4096, 128, 576, 512, 4608
KC = 1024
NC = 512
HR = M // 2
BOUNCE = (960, 960, 960)
EARLY = 6
NBH = sum(BOUNCE) // HR
MF = 512
WO_PIECES = (
    [(h, 0, M) for h in range(10, 18)] + [(h, MF, M - MF) for h in range(24, 32)],
    [(h, 0, M) for h in range(18, 24)],
    [(h, 0, MF) for h in range(24, 28)],
    [(h, 0, MF) for h in range(28, 30)],
    [(30, 0, MF)],
    [(31, 0, MF)],
)
WD_CHUNKS = 3


def _merge(jobs):
    out = []
    for h, r0, n in jobs:
        lo = (h * M + r0) // 2
        if out and out[-1][0] + out[-1][1] == lo:
            out[-1] = (out[-1][0], out[-1][1] + n // 2)
        else:
            out.append((lo, n // 2))
    return out


assert NBH * HR == sum(BOUNCE) and EARLY * HR <= BOUNCE[0] + BOUNCE[1]
assert sum(n for p in WO_PIECES for _, _, n in p) == (H - NBH) * M
N_SEMS = 11 + WD_CHUNKS + sum(len(_merge(p)) for p in WO_PIECES) + 2 * len(BOUNCE)
f32 = jnp.float32
bf16 = jnp.bfloat16
u32 = jnp.uint32


def _dot(a, b):
    return jnp.dot(a, b, preferred_element_type=f32)


def _dot_nt(a, b):
    return lax.dot_general(a, b, (((1,), (1,)), ((), ())), preferred_element_type=f32)


def _iota(shape, dim):
    return lax.broadcasted_iota(jnp.int32, shape, dim)


def _kernel(x_hbm, wr_hbm, wq_hbm, wuk_hbm, ckv_hbm, wuv_hbm, wo_hbm, wg_hbm, wu_hbm, wd_hbm,
            o_ref,
            x_v, wr_v, wq_v, wuk_v, ckv_v, wuv_v, wo_v, wg_v, wu_v, wd_v,
            q_s, qa_s, s_s, cc_s, lc_s, ctx_s, h_s, bounce_sm, sems):
    n_sem = [0]

    def copy(src, dst):
        c = pltpu.make_async_copy(src, dst, sems.at[n_sem[0]])
        n_sem[0] += 1
        return c

    wo32 = wo_hbm.bitcast(u32)

    def wo_copy(row0, nrows):
        return copy(wo32.at[pl.ds(row0, nrows)], wo_v.at[pl.ds(row0, nrows)])

    c_x = copy(x_hbm, x_v)
    c_wr = copy(wr_hbm, wr_v)
    c_wq = copy(wq_hbm.bitcast(u32), wq_v)
    c_wuk = copy(wuk_hbm.bitcast(u32), wuk_v)
    c_ckv = [copy(ckv_hbm.at[b], ckv_v.at[b]) for b in range(B)]
    c_wuv = copy(wuv_hbm.bitcast(u32), wuv_v)
    c_wg = copy(wg_hbm, wg_v)
    c_wu = copy(wu_hbm, wu_v)
    fc = F // WD_CHUNKS
    c_wd = [copy(wd_hbm.at[:, pl.ds(i * fc, fc)], wd_v.at[:, pl.ds(i * fc, fc)])
            for i in range(WD_CHUNKS)]
    c_wo = [[wo_copy(lo, n) for lo, n in _merge(p)] for p in WO_PIECES]
    b_in, b_out, r0 = [], [], 0
    for i, n in enumerate(BOUNCE):
        slot = bounce_sm.at[i % 2, pl.ds(0, n)]
        b_in.append(copy(wo32.at[pl.ds(r0, n)], slot))
        b_out.append(copy(slot, wo_v.at[pl.ds(r0, n)]))
        r0 += n
    assert n_sem[0] == N_SEMS

    for c in [c_x, c_wr, c_wq, b_in[0], b_in[1], c_wuk, *c_ckv, c_wuv, c_wg, c_wu,
              *c_wd]:
        c.start()

    cc_s[...] = jnp.zeros(cc_s.shape, f32)
    ctx_s[pl.ds(4 * H, 8), :] = jnp.zeros((8, D), f32)
    c_x.wait()
    c_wr.wait()
    x = x_v[...].astype(f32)
    x = jnp.concatenate([x, x], axis=0)
    mu = jnp.mean(x, axis=-1, keepdims=True)
    xc = x - mu
    var = jnp.mean(xc * xc, axis=-1, keepdims=True)
    xn = (xc / jnp.sqrt(var + 1e-5)).astype(bf16).astype(f32)
    wr = wr_v[...].astype(f32).reshape(1, M)
    r = jnp.sum(xn * wr, axis=-1, keepdims=True)
    xn8 = xn.astype(bf16)
    E = (_iota((128, 256), 1) // 2 == _iota((128, 256), 0)).astype(f32).astype(bf16)
    ET = (_iota((256, 128), 0) // 2 == _iota((256, 128), 1)).astype(f32).astype(bf16)
    parts = [_dot(xn8[:, 128 * k:128 * (k + 1)], E) for k in range(4)]
    parts.append(_dot(xn8[:, 512:576], E[:64, :128]))
    lx = jnp.concatenate(parts, axis=1)
    lx = jnp.where(_iota((8, 2 * M), 0) // 4 == _iota((8, 2 * M), 1) % 2, lx, 0.0).astype(bf16)

    c_wq.wait()

    def body_q(jj, _):
        ws = [pltpu.bitcast(wq_v[pl.ds(4 * jj + i, M, stride=16), :], bf16) for i in range(4)]
        res = _dot(lx, jnp.concatenate(ws, axis=1)) * (D ** -0.5)
        for i in range(4):
            q_s[pl.ds(pl.multiple_of(8 * (4 * jj + i), 8), 8), :] = res[:, 128 * i:128 * (i + 1)]
        return 0
    lax.fori_loop(0, 4, body_q, 0)
    b_in[0].wait()
    b_out[0].start()

    c_wuk.wait()
    pm = _iota((8, 2 * DC), 0) // 4 == _iota((8, 2 * DC), 1) % 2

    def body_qa(j, _):
        w = pltpu.bitcast(wuk_v[pl.ds(j, DC, stride=16), :], bf16)
        rows = pl.ds(pl.multiple_of(8 * j, 8), 8)
        lc_s[rows, :] = jnp.where(pm, _dot_nt(q_s[rows, :].astype(bf16), w), 0.0)
        return 0
    lax.fori_loop(0, H // 2, body_qa, 0)
    rall = lc_s[...].astype(bf16)
    for k in range(4):
        qa_s[k] = _dot(rall[:, 256 * k:256 * (k + 1)], ET)

    for b in range(B):
        c_ckv[b].wait()
        if b == 2:
            b_in[1].wait()
            b_out[1].start()
            b_out[0].wait()
            b_in[2].start()
        qa = jnp.concatenate([qa_s[k, pl.ds(b, H, stride=4), :] for k in range(4)],
                             axis=1).astype(bf16)

        def body_s(i, mx, b=b, qa=qa):
            s = _dot_nt(qa, ckv_v[b, pl.ds(pl.multiple_of(i * KC, KC), KC), :])
            s_s[i] = s
            for t in range(KC // 128):
                mx = jnp.maximum(mx, s[:, 128 * t:128 * (t + 1)])
            return mx
        mx = lax.fori_loop(0, SK // KC, body_s, jnp.full((H, 128), -jnp.inf, f32))
        mx = jnp.max(mx, axis=1, keepdims=True)

        def body_pv(i, carry, b=b, mx=mx):
            acc, l = carry
            p = jnp.exp(s_s[i] - mx)
            for t in range(KC // 128):
                l = l + p[:, 128 * t:128 * (t + 1)]
            kk = ckv_v[b, pl.ds(pl.multiple_of(i * KC, KC), KC), :]
            return acc + _dot(p.astype(bf16), kk), l
        acc, l = lax.fori_loop(0, SK // KC, body_pv,
                               (jnp.zeros((H, DC), f32), jnp.zeros((H, 128), f32)))
        acc = acc / jnp.sum(l, axis=1, keepdims=True)
        for k in range(4):
            cc_s[k, pl.ds(b, H, stride=4), :] = acc[:, 128 * k:128 * (k + 1)]

    c_wuv.wait()
    pm2 = (_iota((128, 256), 0) // 4) % 2 == _iota((128, 256), 1) % 2
    for k in range(4):
        lc_s[:, 256 * k:256 * (k + 1)] = jnp.where(pm2, _dot(cc_s[k].astype(bf16), E), 0.0)

    def body_ctx(j, _):
        w = pltpu.bitcast(wuv_v[pl.ds(j, DC, stride=16), :], bf16)
        rows = pl.ds(pl.multiple_of(8 * j, 8), 8)
        ctx_s[rows, :] = _dot(lc_s[rows, :].astype(bf16), w)
        return 0
    lax.fori_loop(0, H // 2, body_ctx, 0)

    c_wg.wait()

    def body_g(i, _):
        cols = pl.ds(pl.multiple_of(i * NC, NC), NC)
        h_s[:, cols] = _dot(xn8, wg_v[:, cols])
        return 0
    lax.fori_loop(0, F // NC, body_g, 0)
    b_in[2].wait()
    b_out[2].start()
    c_wu.wait()
    for c in [c for p in c_wo for c in p]:
        c.start()

    def body_u(i, _):
        cols = pl.ds(pl.multiple_of(i * NC, NC), NC)
        g = h_s[:, cols]
        h_s[:, cols] = g * jax.nn.sigmoid(g) * _dot(xn8, wu_v[:, cols])
        return 0
    lax.fori_loop(0, F // NC, body_u, 0)

    def o_jobs(jobs, lo, hi):
        for h, r0, n in jobs:
            w = pltpu.bitcast(wo_v[pl.ds((h * M + r0) // 2, n // 2), :], bf16)
            res = _dot_nt(ctx_s[pl.ds(4 * h, 8), :].astype(bf16), w)
            if r0 == 0:
                lo = lo + res[:, :MF]
            if r0 + n == M:
                hi = hi + res[:, n - (M - MF):]
        return lo, hi

    b_out[1].wait()
    s_lo, s_hi = o_jobs([(h, 0, M) for h in range(EARLY)],
                        jnp.zeros((8, MF), f32), jnp.zeros((8, M - MF), f32))

    def body_d(i, y):
        cols = pl.ds(pl.multiple_of(i * NC, NC), NC)
        return y + _dot_nt(h_s[:, cols].astype(bf16), wd_v[:, cols])
    y = jnp.zeros((8, M), f32)
    for i in range(WD_CHUNKS):
        c_wd[i].wait()
        y = lax.fori_loop(i * (fc // NC), (i + 1) * (fc // NC), body_d, y)
    t = xn + y * jax.nn.sigmoid(r)
    gate = t * jax.nn.sigmoid(t)

    for i, (cs, jobs) in enumerate(zip(c_wo[:-1], WO_PIECES[:-1])):
        for c in cs:
            c.wait()
        s_lo, s_hi = o_jobs(jobs, s_lo, s_hi)
        if i == 0:
            b_out[2].wait()
            s_lo, s_hi = o_jobs([(h, 0, M) for h in range(EARLY, NBH)], s_lo, s_hi)
        if i == 1:
            o_ref[:, MF:] = (x[:, MF:] + s_hi * gate[:, MF:]).astype(bf16)[:B]
    base = x[:, :MF] + s_lo * gate[:, :MF]
    c_last = ctx_s[pl.ds(4 * (H - 1), 8), :].astype(bf16)
    c_wo[-1][0].wait()
    w = pltpu.bitcast(wo_v[pl.ds((H - 1) * HR, MF // 2), :], bf16)
    o_ref[:, :MF] = (base + _dot_nt(c_last, w) * gate[:, :MF]).astype(bf16)[:B]


@jax.jit
def pallas_recurrent_scan__compressed_kv_cla__moe_arch_mod__decode_kernel(
    A_x: jax.Array,
    A_c_kv: jax.Array,
    A_w_q: jax.Array,
    A_w_uk: jax.Array,
    A_w_uv: jax.Array,
    A_w_o: jax.Array,
    B_x: jax.Array,
    B_w_r: jax.Array,
    B_w_gate: jax.Array,
    B_w_up: jax.Array,
    B_w_down: jax.Array,
):
    del B_x
    x = A_x.reshape(B, M)
    wq = A_w_q.reshape(M * H, D)
    wuk = A_w_uk.reshape(DC * H, D)
    wuv = A_w_uv.reshape(DC * H, D)
    wo = jnp.transpose(A_w_o, (0, 2, 1)).reshape(H * M, D)
    wd = B_w_down.T
    out = pl.pallas_call(
        _kernel,
        out_shape=jax.ShapeDtypeStruct((B, M), bf16),
        in_specs=[pl.BlockSpec(memory_space=pl.ANY)] * 10,
        out_specs=pl.BlockSpec(memory_space=pltpu.VMEM),
        scratch_shapes=[
            pltpu.VMEM((B, M), bf16),
            pltpu.VMEM((M,), bf16),
            pltpu.VMEM((M * H // 2, D), u32),
            pltpu.VMEM((DC * H // 2, D), u32),
            pltpu.VMEM((B, SK, DC), bf16),
            pltpu.VMEM((DC * H // 2, D), u32),
            pltpu.VMEM((H * HR, D), u32),
            pltpu.VMEM((M, F), bf16),
            pltpu.VMEM((M, F), bf16),
            pltpu.VMEM((M, F), bf16),
            pltpu.VMEM((128, 128), f32),
            pltpu.VMEM((4, 128, 128), f32),
            pltpu.VMEM((SK // KC, H, KC), f32),
            pltpu.VMEM((4, 128, 128), f32),
            pltpu.VMEM((128, 2 * DC), f32),
            pltpu.VMEM((4 * H + 8, D), f32),
            pltpu.VMEM((8, F), f32),
            pltpu.SMEM((2, max(BOUNCE), D), u32),
            pltpu.SemaphoreType.DMA((N_SEMS,)),
        ],
        compiler_params=pltpu.CompilerParams(
            vmem_limit_bytes=100 * 1024 * 1024,
            disable_semaphore_checks=True,
        ),
    )(x, B_w_r, wq, wuk, A_c_kv, wuv, wo, B_w_gate, B_w_up, wd)
    return out.reshape(B, 1, M)
```

```python
import jax
import jax.numpy as jnp
from jax import lax
from jax.experimental import pallas as pl
from jax.experimental.pallas import tpu as pltpu

B, H, SK, D, M, DC, F = 4, 32, 4096, 128, 576, 512, 4608
KC = 1024
NC = 512
HR = M // 2
MF = 512
G = 8
SHIFT = 6
LOOKAHEAD = 6
f32 = jnp.float32
bf16 = jnp.bfloat16
u32 = jnp.uint32


def _dot(a, b):
    return jnp.dot(a, b, preferred_element_type=f32)


def _dot_nt(a, b):
    return lax.dot_general(a, b, (((1,), (1,)), ((), ())), preferred_element_type=f32)


def _iota(shape, dim):
    return lax.broadcasted_iota(jnp.int32, shape, dim)


def _mul(k, c):
    return k * c if isinstance(k, int) else pl.multiple_of(k * c, c)


def _kernel(x_hbm, wr_hbm, wq_hbm, wuk_hbm, ckv_hbm, wuv_hbm, wo_hbm, wg_hbm, wu_hbm, wd_hbm,
            o_ref,
            x_v, wr_v, wq_v, wuk_v, ckv_v, wuv_v, wo_v, wg_v, wu_v, wd_v,
            q_s, qa_s, s_s, cc_s, lc_s, ctx_s, h_s, sems):
    wo32 = wo_hbm.bitcast(u32)

    def rows_unit(src, dst, row0, region_rows, r):
        def view(g, k):
            rows = pl.ds(row0 + g * region_rows + _mul(k, r), r)
            return src.at[rows], dst.at[rows]
        return view

    def ffn_unit(src, dst):
        def view(g, k):
            rows = pl.ds(g * (M // G) + _mul(k // 2, 8), 8)
            cols = pl.ds(_mul(k % 2, F // 2), F // 2)
            return src.at[rows, cols], dst.at[rows, cols]
        return view

    units = [('wq', 16, rows_unit(wq_hbm.bitcast(u32), wq_v, 0, 1152, 72)),
             ('wuk', 16, rows_unit(wuk_hbm.bitcast(u32), wuk_v, 0, 1024, 64))]
    for b in range(B):
        units.append((f'ckv{b}', 16, rows_unit(ckv_hbm.at[b], ckv_v.at[b], 0, 512, 32)))
    units += [('wuv', 16, rows_unit(wuv_hbm.bitcast(u32), wuv_v, 0, 1024, 64)),
              ('wg', 18, ffn_unit(wg_hbm, wg_v)),
              ('wu', 18, ffn_unit(wu_hbm, wu_v)),
              ('wd', 18, ffn_unit(wd_hbm, wd_v)),
              ('wo0', 8, rows_unit(wo32, wo_v, 0, 2 * HR, 72)),
              ('woh', 1, rows_unit(wo32, wo_v, 24 * HR + MF // 2, HR, 32)),
              ('wo1', 4, rows_unit(wo32, wo_v, 16 * HR, HR, 72))]
    tail = [(f'wt{h}', 1, (lambda g, k, h=h: (wo32.at[pl.ds(h * HR + 64 * (g // 2), 64)],
                                                wo_v.at[pl.ds(h * HR + 64 * (g // 2), 64)])))
            for h in range(24, 32)]
    sem_of = {}
    for name, _, _ in units + tail:
        sem_of[name] = len(sem_of) + 2
    rounds_a = [(u, k) for u in units for k in range(u[1])]
    rounds_b = rounds_a + [(u, 0) for u in tail]
    end = {}
    n = 0
    for u in units:
        n += u[1]
        end[u[0]] = n
    NR = n
    last = len(rounds_b) - SHIFT

    def start(u, g, k):
        src, dst = u[2](g, k)
        pltpu.make_async_copy(src, dst, sems.at[sem_of[u[0]]]).start(priority=g % 2)

    def issue(ua, ka, ub, kb):
        for j in range(G // 2):
            if ub is not None:
                start(ub, 2 * j + 1, kb)
            if ua is not None:
                start(ua, 2 * j, ka)

    def at(rho):
        a = rounds_a[rho] if 0 <= rho < NR else (None, 0)
        b_ = rounds_b[rho + SHIFT] if rho + SHIFT < len(rounds_b) else (None, 0)
        return a, b_

    def runs(lo, hi):
        out = []
        for rho in range(lo, hi):
            (ua, ka), (ub, kb) = at(rho)
            if out and out[-1][2] is ua and out[-1][4] is ub:
                out[-1][1] += 1
            else:
                out.append([rho, 1, ua, ka, ub, kb])
        return out

    pos = [-SHIFT]

    def issue_upto(target):
        target = min(target, last)
        for _, cnt, ua, ka, ub, kb in runs(pos[0], target):
            if cnt == 1:
                issue(ua, ka, ub, kb)
            else:
                def body(i, _, ua=ua, ka=ka, ub=ub, kb=kb):
                    issue(ua, ka + i, ub, kb + i)
                    return 0
                lax.fori_loop(0, cnt, body, 0)
        pos[0] = max(pos[0], target)

    def paced(plan):
        cnt, step = plan
        rs = runs(pos[0], min(pos[0] + cnt, last))
        p0 = pos[0]
        pos[0] = min(pos[0] + cnt, last)

        def fn(i):
            for rho0, c, ua, ka, ub, kb in rs:
                lo = rho0 - p0
                cond = jnp.logical_and(i >= lo * step, i < (lo + c) * step)
                if step > 1:
                    cond = jnp.logical_and(cond, i % step == 0)

                @pl.when(cond)
                def _(ua=ua, ka=ka, ub=ub, kb=kb, lo=lo, c=c):
                    t = i // step - lo if c > 1 else 0
                    issue(ua, ka + t, ub, kb + t)
        return fn

    def wait(name, *bufs):
        if name in end:
            issue_upto(end[name] + LOOKAHEAD)
        for buf in bufs:
            pltpu.make_async_copy(buf, buf, sems.at[sem_of[name]]).wait()

    c_x = pltpu.make_async_copy(x_hbm, x_v, sems.at[0])
    c_wr = pltpu.make_async_copy(wr_hbm, wr_v, sems.at[1])
    issue_upto(-SHIFT + 1)
    c_x.start()
    c_wr.start()
    issue_upto(5)

    cc_s[...] = jnp.zeros(cc_s.shape, f32)
    ctx_s[pl.ds(4 * H, 8), :] = jnp.zeros((8, D), f32)
    c_x.wait()
    c_wr.wait()
    x = x_v[...].astype(f32)
    x = jnp.concatenate([x, x], axis=0)
    mu = jnp.mean(x, axis=-1, keepdims=True)
    xc = x - mu
    var = jnp.mean(xc * xc, axis=-1, keepdims=True)
    xn = (xc / jnp.sqrt(var + 1e-5)).astype(bf16).astype(f32)
    wr = wr_v[...].astype(f32).reshape(1, M)
    r = jnp.sum(xn * wr, axis=-1, keepdims=True)
    xn8 = xn.astype(bf16)
    E = (_iota((128, 256), 1) // 2 == _iota((128, 256), 0)).astype(f32).astype(bf16)
    ET = (_iota((256, 128), 0) // 2 == _iota((256, 128), 1)).astype(f32).astype(bf16)
    parts = [_dot(xn8[:, 128 * k:128 * (k + 1)], E) for k in range(4)]
    parts.append(_dot(xn8[:, 512:576], E[:64, :128]))
    lx = jnp.concatenate(parts, axis=1)
    lx = jnp.where(_iota((8, 2 * M), 0) // 4 == _iota((8, 2 * M), 1) % 2, lx, 0.0).astype(bf16)

    wait('wq', wq_v)
    pace = paced((8, 1))

    def body_q(jj, _):
        pace(jj)
        ws = [pltpu.bitcast(wq_v[pl.ds(2 * jj + i, M, stride=16), :], bf16) for i in range(2)]
        res = _dot(lx, jnp.concatenate(ws, axis=1)) * (D ** -0.5)
        for i in range(2):
            q_s[pl.ds(pl.multiple_of(8 * (2 * jj + i), 8), 8), :] = res[:, 128 * i:128 * (i + 1)]
        return 0
    lax.fori_loop(0, 8, body_q, 0)

    wait('wuk', wuk_v)
    pm = _iota((8, 2 * DC), 0) // 4 == _iota((8, 2 * DC), 1) % 2
    pace = paced((14, 1))

    def body_qa(j, _):
        pace(j)
        w = pltpu.bitcast(wuk_v[pl.ds(j, DC, stride=16), :], bf16)
        rows = pl.ds(pl.multiple_of(8 * j, 8), 8)
        lc_s[rows, :] = jnp.where(pm, _dot_nt(q_s[rows, :].astype(bf16), w), 0.0)
        return 0
    lax.fori_loop(0, H // 2, body_qa, 0)
    rall = lc_s[...].astype(bf16)
    for k in range(4):
        qa_s[k] = _dot(rall[:, 256 * k:256 * (k + 1)], ET)

    for b in range(B):
        wait(f'ckv{b}', ckv_v.at[b])
        qa = jnp.concatenate([qa_s[k, pl.ds(b, H, stride=4), :] for k in range(4)],
                             axis=1).astype(bf16)
        pace = paced((4, 1))

        def body_s(i, mx, b=b, qa=qa, pace=pace):
            pace(i)
            s = _dot_nt(qa, ckv_v[b, pl.ds(pl.multiple_of(i * KC, KC), KC), :])
            s_s[i] = s
            for t in range(KC // 128):
                mx = jnp.maximum(mx, s[:, 128 * t:128 * (t + 1)])
            return mx
        mx = lax.fori_loop(0, SK // KC, body_s, jnp.full((H, 128), -jnp.inf, f32))
        mx = jnp.max(mx, axis=1, keepdims=True)
        pace = paced((4, 1))

        def body_pv(i, carry, b=b, mx=mx, pace=pace):
            pace(i)
            acc, l = carry
            p = jnp.exp(s_s[i] - mx)
            for t in range(KC // 128):
                l = l + p[:, 128 * t:128 * (t + 1)]
            kk = ckv_v[b, pl.ds(pl.multiple_of(i * KC, KC), KC), :]
            return acc + _dot(p.astype(bf16), kk), l
        acc, l = lax.fori_loop(0, SK // KC, body_pv,
                               (jnp.zeros((H, DC), f32), jnp.zeros((H, 128), f32)))
        acc = acc / jnp.sum(l, axis=1, keepdims=True)
        for k in range(4):
            cc_s[k, pl.ds(b, H, stride=4), :] = acc[:, 128 * k:128 * (k + 1)]

    wait('wuv', wuv_v)
    pm2 = (_iota((128, 256), 0) // 4) % 2 == _iota((128, 256), 1) % 2
    for k in range(4):
        lc_s[:, 256 * k:256 * (k + 1)] = jnp.where(pm2, _dot(cc_s[k].astype(bf16), E), 0.0)
    pace = paced((14, 1))

    def body_ctx(j, _):
        pace(j)
        w = pltpu.bitcast(wuv_v[pl.ds(j, DC, stride=16), :], bf16)
        rows = pl.ds(pl.multiple_of(8 * j, 8), 8)
        ctx_s[rows, :] = _dot(lc_s[rows, :].astype(bf16), w)
        return 0
    lax.fori_loop(0, H // 2, body_ctx, 0)

    wait('wg', wg_v)
    pace = paced((5, 2))

    def body_g(i, _):
        pace(i)
        cols = pl.ds(pl.multiple_of(i * NC, NC), NC)
        h_s[:, cols] = _dot(xn8, wg_v[:, cols])
        return 0
    lax.fori_loop(0, F // NC, body_g, 0)
    wait('wu', wu_v)
    pace = paced((5, 2))

    def body_u(i, _):
        pace(i)
        cols = pl.ds(pl.multiple_of(i * NC, NC), NC)
        g = h_s[:, cols]
        h_s[:, cols] = g * jax.nn.sigmoid(g) * _dot(xn8, wu_v[:, cols])
        return 0
    lax.fori_loop(0, F // NC, body_u, 0)

    wait('wd', wd_v)
    pace = paced((8, 1))

    def body_d(i, y):
        pace(i)
        cols = pl.ds(pl.multiple_of(i * NC, NC), NC)
        return y + _dot_nt(h_s[:, cols].astype(bf16), wd_v[:, cols])
    y = lax.fori_loop(0, F // NC, body_d, jnp.zeros((8, M), f32))
    t = xn + y * jax.nn.sigmoid(r)
    gate = t * jax.nn.sigmoid(t)

    def o_jobs(jobs, lo, hi):
        for h, r0, n in jobs:
            w = pltpu.bitcast(wo_v[pl.ds((h * M + r0) // 2, n // 2), :], bf16)
            res = _dot_nt(ctx_s[pl.ds(4 * h, 8), :].astype(bf16), w)
            if r0 == 0:
                lo = lo + res[:, :MF]
            if r0 + n == M:
                hi = hi + res[:, n - (M - MF):]
        return lo, hi

    issue_upto(last)
    wait('wo0', wo_v.at[pl.ds(0, 16 * HR)])
    s_lo, s_hi = o_jobs([(h, 0, M) for h in range(16)], jnp.zeros((8, MF), f32), jnp.zeros((8, M - MF), f32))
    wait('woh', *[wo_v.at[pl.ds(h * HR + MF // 2, HR - MF // 2)] for h in range(24, 32)])
    wait('wo1', wo_v.at[pl.ds(16 * HR, 8 * HR)])
    s_lo, s_hi = o_jobs([(h, 0, M) for h in range(16, 24)] + [(h, MF, M - MF) for h in range(24, 32)], s_lo, s_hi)
    o_ref[:, MF:] = (x[:, MF:] + s_hi * gate[:, MF:]).astype(bf16)[:B]
    for hs in ((24, 25, 26, 27), (28, 29), (30,)):
        for h in hs:
            wait(f'wt{h}', wo_v.at[pl.ds(h * HR, MF // 2)])
        s_lo, s_hi = o_jobs([(h, 0, MF) for h in hs], s_lo, s_hi)
    base = x[:, :MF] + s_lo * gate[:, :MF]
    c_last = ctx_s[pl.ds(4 * (H - 1), 8), :].astype(bf16)
    wait('wt31', wo_v.at[pl.ds(31 * HR, MF // 2)])
    w = pltpu.bitcast(wo_v[pl.ds((H - 1) * HR, MF // 2), :], bf16)
    o_ref[:, :MF] = (base + _dot_nt(c_last, w) * gate[:, :MF]).astype(bf16)[:B]
    assert pos[0] == last


@jax.jit
def pallas_recurrent_scan__compressed_kv_cla__moe_arch_mod__decode_kernel(
    A_x: jax.Array,
    A_c_kv: jax.Array,
    A_w_q: jax.Array,
    A_w_uk: jax.Array,
    A_w_uv: jax.Array,
    A_w_o: jax.Array,
    B_x: jax.Array,
    B_w_r: jax.Array,
    B_w_gate: jax.Array,
    B_w_up: jax.Array,
    B_w_down: jax.Array,
):
    del B_x
    x = A_x.reshape(B, M)
    wq = A_w_q.reshape(M * H, D)
    wuk = A_w_uk.reshape(DC * H, D)
    wuv = A_w_uv.reshape(DC * H, D)
    wo = jnp.transpose(A_w_o, (0, 2, 1)).reshape(H * M, D)
    wd = B_w_down.T
    out = pl.pallas_call(
        _kernel,
        out_shape=jax.ShapeDtypeStruct((B, M), bf16),
        in_specs=[pl.BlockSpec(memory_space=pl.ANY)] * 10,
        out_specs=pl.BlockSpec(memory_space=pltpu.VMEM),
        scratch_shapes=[
            pltpu.VMEM((B, M), bf16),
            pltpu.VMEM((M,), bf16),
            pltpu.VMEM((M * H // 2, D), u32),
            pltpu.VMEM((DC * H // 2, D), u32),
            pltpu.VMEM((B, SK, DC), bf16),
            pltpu.VMEM((DC * H // 2, D), u32),
            pltpu.VMEM((H * HR, D), u32),
            pltpu.VMEM((M, F), bf16),
            pltpu.VMEM((M, F), bf16),
            pltpu.VMEM((M, F), bf16),
            pltpu.VMEM((128, 128), f32),
            pltpu.VMEM((4, 128, 128), f32),
            pltpu.VMEM((SK // KC, H, KC), f32),
            pltpu.VMEM((4, 128, 128), f32),
            pltpu.VMEM((128, 2 * DC), f32),
            pltpu.VMEM((4 * H + 8, D), f32),
            pltpu.VMEM((8, F), f32),
            pltpu.SemaphoreType.DMA((2 + 13 + 8,)),
        ],
        compiler_params=pltpu.CompilerParams(
            vmem_limit_bytes=100 * 1024 * 1024,
            disable_semaphore_checks=True,
            disable_bounds_checks=True,
        ),
    )(x, B_w_r, wq, wuk, A_c_kv, wuv, wo, B_w_gate, B_w_up, wd)
    return out.reshape(B, 1, M)
```

```python
import jax
import jax.numpy as jnp
from jax import lax
from jax.experimental import pallas as pl
from jax.experimental.pallas import tpu as pltpu

B, H, SK, D, M, DC, F = 4, 32, 4096, 128, 576, 512, 4608
KC = 1024
NC = 512
HR = M // 2
MF = 512
G = 8
SHIFT = 6
LOOKAHEAD = 6
TAIL = tuple(range(3, H, 4))
N_SEMS = 2 + 11 + len(TAIL)
f32 = jnp.float32
bf16 = jnp.bfloat16
u32 = jnp.uint32


def _dot(a, b):
    return jnp.dot(a, b, preferred_element_type=f32)


def _dot_nt(a, b):
    return lax.dot_general(a, b, (((1,), (1,)), ((), ())), preferred_element_type=f32)


def _iota(shape, dim):
    return lax.broadcasted_iota(jnp.int32, shape, dim)


def _mul(k, c):
    return k * c if isinstance(k, int) else pl.multiple_of(k * c, c)


def _kernel(x_hbm, wr_hbm, wq_hbm, wuk_hbm, ckv_hbm, wuv_hbm, wo_hbm, wg_hbm, wu_hbm, wd_hbm,
            o_ref,
            x_v, wr_v, wq_v, wuk_v, ckv_v, wuv_v, wo_v, wg_v, wu_v, wd_v,
            q_s, qa_s, s_s, cc_s, lc_s, ctx_s, h_s, sems):
    def rows_unit(src, dst, row0, region_rows, r):
        def view(g, k):
            rows = pl.ds(row0 + g * region_rows + _mul(k, r), r)
            return src.at[rows], dst.at[rows]
        return view

    def ffn_unit(src, dst):
        def view(g, k):
            rows = pl.ds(g * (M // G) + _mul(k // 2, 8), 8)
            cols = pl.ds(_mul(k % 2, F // 2), F // 2)
            return src.at[rows, cols], dst.at[rows, cols]
        return view

    wo32 = wo_hbm.bitcast(u32)
    units = [('wq', 16, rows_unit(wq_hbm.bitcast(u32), wq_v, 0, 1152, 72)),
             ('wuk', 16, rows_unit(wuk_hbm.bitcast(u32), wuk_v, 0, 1024, 64)),
             ('ckv0', 32, rows_unit(ckv_hbm.at[0], ckv_v.at[0], 0, 1024, 32)),
             ('ckv1', 32, rows_unit(ckv_hbm.at[1], ckv_v.at[1], 0, 1024, 32)),
             ('wuv', 16, rows_unit(wuv_hbm.bitcast(u32), wuv_v, 0, 1024, 64)),
             ('wg', 18, ffn_unit(wg_hbm, wg_v)),
             ('wu', 18, ffn_unit(wu_hbm, wu_v)),
             ('wd', 18, ffn_unit(wd_hbm, wd_v)),
             ('wo0', 8, rows_unit(wo32, wo_v, 0, 4 * HR, 72)),
             ('woh', 1, rows_unit(wo32, wo_v, 3 * HR + MF // 2, 4 * HR, 32)),
             ('wo1', 4, rows_unit(wo32, wo_v, 2 * HR, 4 * HR, 72))]
    tail = [(f'wt{h}', 1, rows_unit(wo32, wo_v, h * HR - 32, 32, 64)) for h in TAIL]
    sem_of = {u[0]: i + 2 for i, u in enumerate(units + tail)}
    assert len(sem_of) + 2 == N_SEMS
    rounds_a = [(u, k) for u in units for k in range(u[1])]
    rounds_b = rounds_a + [(u, 0) for u in tail]
    end = {u[0]: i + 1 for i, (u, _) in enumerate(rounds_a)}
    last = len(rounds_b) - SHIFT
    pos = [-SHIFT]

    def issue(ua, ka, ub, kb):
        for g in range(0, G, 2):
            for u, k, p in ((ub, kb, 1), (ua, ka, 0)):
                if u is not None:
                    src, dst = u[2](g + p, k)
                    pltpu.make_async_copy(src, dst, sems.at[sem_of[u[0]]]).start(priority=p)

    def take(n):
        lo, hi = pos[0], max(pos[0], min(pos[0] + n, last))
        pos[0] = hi
        out = []
        for rho in range(lo, hi):
            ua, ka = rounds_a[rho] if 0 <= rho < len(rounds_a) else (None, 0)
            ub, kb = rounds_b[rho + SHIFT]
            if out and out[-1][2] is ua and out[-1][4] is ub:
                out[-1][1] += 1
            else:
                out.append([rho - lo, 1, ua, ka, ub, kb])
        return out

    def issue_next(n):
        for _, cnt, ua, ka, ub, kb in take(n):
            if cnt == 1:
                issue(ua, ka, ub, kb)
            else:
                def body(i, _, ua=ua, ka=ka, ub=ub, kb=kb):
                    issue(ua, ka + i, ub, kb + i)
                    return 0
                lax.fori_loop(0, cnt, body, 0)

    def paced_loop(trips, n, step, body, init):
        assert (n - 1) * step < trips
        runs = take(n)

        def wrapped(i, carry):
            for lo, cnt, ua, ka, ub, kb in runs:
                cond = jnp.logical_and(i >= lo * step, i < (lo + cnt) * step)
                if step > 1:
                    cond = jnp.logical_and(cond, i % step == 0)

                @pl.when(cond)
                def _(lo=lo, cnt=cnt, ua=ua, ka=ka, ub=ub, kb=kb):
                    t = jnp.clip(i // step - lo, 0, cnt - 1) if cnt > 1 else 0
                    issue(ua, ka + t, ub, kb + t)
            return body(i, carry)
        return lax.fori_loop(0, trips, wrapped, init)

    def wait(name, *bufs):
        if name in end:
            issue_next(end[name] + LOOKAHEAD - pos[0])
        for buf in bufs:
            pltpu.make_async_copy(buf, buf, sems.at[sem_of[name]]).wait()

    c_x = pltpu.make_async_copy(x_hbm, x_v, sems.at[0])
    c_wr = pltpu.make_async_copy(wr_hbm, wr_v, sems.at[1])
    issue_next(1)
    c_x.start()
    c_wr.start()
    issue_next(SHIFT + 4)

    cc_s[...] = jnp.zeros(cc_s.shape, f32)
    ctx_s[pl.ds(4 * H, 8), :] = jnp.zeros((8, D), f32)
    c_x.wait()
    c_wr.wait()
    x = x_v[...].astype(f32)
    x = jnp.concatenate([x, x], axis=0)
    mu = jnp.mean(x, axis=-1, keepdims=True)
    xc = x - mu
    var = jnp.mean(xc * xc, axis=-1, keepdims=True)
    xn = (xc / jnp.sqrt(var + 1e-5)).astype(bf16).astype(f32)
    wr = wr_v[...].astype(f32).reshape(1, M)
    r = jnp.sum(xn * wr, axis=-1, keepdims=True)
    xn8 = xn.astype(bf16)
    E = (_iota((128, 256), 1) // 2 == _iota((128, 256), 0)).astype(f32).astype(bf16)
    ET = (_iota((256, 128), 0) // 2 == _iota((256, 128), 1)).astype(f32).astype(bf16)
    parts = [_dot(xn8[:, 128 * k:128 * (k + 1)], E) for k in range(4)]
    parts.append(_dot(xn8[:, 512:576], E[:64, :128]))
    lx = jnp.concatenate(parts, axis=1)
    lx = jnp.where(_iota((8, 2 * M), 0) // 4 == _iota((8, 2 * M), 1) % 2, lx, 0.0).astype(bf16)

    wait('wq', wq_v)

    def body_q(jj, _):
        ws = [pltpu.bitcast(wq_v[pl.ds(2 * jj + i, M, stride=16), :], bf16) for i in range(2)]
        res = _dot(lx, jnp.concatenate(ws, axis=1)) * (D ** -0.5)
        for i in range(2):
            q_s[pl.ds(pl.multiple_of(8 * (2 * jj + i), 8), 8), :] = res[:, 128 * i:128 * (i + 1)]
        return 0
    paced_loop(8, 8, 1, body_q, 0)
    issue_next(2)

    wait('wuk', wuk_v)
    pm = _iota((8, 2 * DC), 0) // 4 == _iota((8, 2 * DC), 1) % 2

    def body_qa(j, _):
        w = pltpu.bitcast(wuk_v[pl.ds(j, DC, stride=16), :], bf16)
        rows = pl.ds(pl.multiple_of(8 * j, 8), 8)
        lc_s[rows, :] = jnp.where(pm, _dot_nt(q_s[rows, :].astype(bf16), w), 0.0)
        return 0
    paced_loop(H // 2, 14, 1, body_qa, 0)
    rall = lc_s[...].astype(bf16)
    for k in range(4):
        qa_s[k] = _dot(rall[:, 256 * k:256 * (k + 1)], ET)

    for b in range(B):
        if b % 2 == 0:
            wait(f'ckv{b // 2}', ckv_v.at[b // 2])
        kv = ckv_v.at[b // 2, pl.ds((b % 2) * SK, SK)]
        qa = jnp.concatenate([qa_s[k, pl.ds(b, H, stride=4), :] for k in range(4)],
                             axis=1).astype(bf16)

        def body_s(i, mx, kv=kv, qa=qa):
            s = _dot_nt(qa, kv[pl.ds(pl.multiple_of(i * KC, KC), KC), :])
            s_s[i] = s
            for t in range(KC // 128):
                mx = jnp.maximum(mx, s[:, 128 * t:128 * (t + 1)])
            return mx
        mx = paced_loop(SK // KC, 4, 1, body_s, jnp.full((H, 128), -jnp.inf, f32))
        issue_next(1)
        mx = jnp.max(mx, axis=1, keepdims=True)

        def body_pv(i, carry, kv=kv, mx=mx):
            acc, l = carry
            p = jnp.exp(s_s[i] - mx)
            for t in range(KC // 128):
                l = l + p[:, 128 * t:128 * (t + 1)]
            kk = kv[pl.ds(pl.multiple_of(i * KC, KC), KC), :]
            return acc + _dot(p.astype(bf16), kk), l
        acc, l = paced_loop(SK // KC, 4, 1, body_pv,
                            (jnp.zeros((H, DC), f32), jnp.zeros((H, 128), f32)))
        acc = acc / jnp.sum(l, axis=1, keepdims=True)
        for k in range(4):
            cc_s[k, pl.ds(b, H, stride=4), :] = acc[:, 128 * k:128 * (k + 1)]

    wait('wuv', wuv_v)
    pm2 = (_iota((128, 256), 0) // 4) % 2 == _iota((128, 256), 1) % 2
    for k in range(4):
        lc_s[:, 256 * k:256 * (k + 1)] = jnp.where(pm2, _dot(cc_s[k].astype(bf16), E), 0.0)

    def body_ctx(j, _):
        w = pltpu.bitcast(wuv_v[pl.ds(j, DC, stride=16), :], bf16)
        rows = pl.ds(pl.multiple_of(8 * j, 8), 8)
        ctx_s[rows, :] = _dot(lc_s[rows, :].astype(bf16), w)
        return 0
    issue_next(1)
    paced_loop(H // 2, 14, 1, body_ctx, 0)

    wait('wg', wg_v)

    def body_g(i, _):
        cols = pl.ds(pl.multiple_of(i * NC, NC), NC)
        h_s[:, cols] = _dot(xn8, wg_v[:, cols])
        return 0
    paced_loop(F // NC, 5, 2, body_g, 0)
    wait('wu', wu_v)

    def body_u(i, _):
        cols = pl.ds(pl.multiple_of(i * NC, NC), NC)
        g = h_s[:, cols]
        h_s[:, cols] = g * jax.nn.sigmoid(g) * _dot(xn8, wu_v[:, cols])
        return 0
    paced_loop(F // NC, 5, 2, body_u, 0)

    wait('wd', wd_v)

    def body_d(i, y):
        cols = pl.ds(pl.multiple_of(i * NC, NC), NC)
        return y + _dot_nt(h_s[:, cols].astype(bf16), wd_v[:, cols])
    y = paced_loop(F // NC, 8, 1, body_d, jnp.zeros((8, M), f32))
    t = xn + y * jax.nn.sigmoid(r)
    gate = t * jax.nn.sigmoid(t)

    def o_jobs(jobs, lo, hi):
        for h, r0, n in jobs:
            w = pltpu.bitcast(wo_v[pl.ds((h * M + r0) // 2, n // 2), :], bf16)
            res = _dot_nt(ctx_s[pl.ds(4 * h, 8), :].astype(bf16), w)
            if r0 == 0:
                lo = lo + res[:, :MF]
            if r0 + n == M:
                hi = hi + res[:, n - (M - MF):]
        return lo, hi

    issue_next(last - pos[0])
    wait('wo0', *[wo_v.at[pl.ds(4 * g * HR, 2 * HR)] for g in range(G)])
    s_lo, s_hi = o_jobs([(h, 0, M) for h in range(H) if h % 4 < 2],
                        jnp.zeros((8, MF), f32), jnp.zeros((8, M - MF), f32))
    wait('woh', *[wo_v.at[pl.ds(h * HR + MF // 2, HR - MF // 2)] for h in TAIL])
    wait('wo1', *[wo_v.at[pl.ds(h * HR, HR)] for h in range(2, H, 4)])
    s_lo, s_hi = o_jobs([(h, 0, M) for h in range(2, H, 4)] + [(h, MF, M - MF) for h in TAIL],
                        s_lo, s_hi)
    o_ref[:, MF:] = (x[:, MF:] + s_hi * gate[:, MF:]).astype(bf16)[:B]
    for hs in (TAIL[:4], TAIL[4:6], TAIL[6:7]):
        for h in hs:
            wait(f'wt{h}', wo_v.at[pl.ds(h * HR, MF // 2)])
        s_lo, s_hi = o_jobs([(h, 0, MF) for h in hs], s_lo, s_hi)
    base = x[:, :MF] + s_lo * gate[:, :MF]
    c_last = ctx_s[pl.ds(4 * (H - 1), 8), :].astype(bf16)
    wait(f'wt{H - 1}', wo_v.at[pl.ds((H - 1) * HR, MF // 2)])
    w = pltpu.bitcast(wo_v[pl.ds((H - 1) * HR, MF // 2), :], bf16)
    o_ref[:, :MF] = (base + _dot_nt(c_last, w) * gate[:, :MF]).astype(bf16)[:B]


@jax.jit
def pallas_recurrent_scan__compressed_kv_cla__moe_arch_mod__decode_kernel(
    A_x: jax.Array,
    A_c_kv: jax.Array,
    A_w_q: jax.Array,
    A_w_uk: jax.Array,
    A_w_uv: jax.Array,
    A_w_o: jax.Array,
    B_x: jax.Array,
    B_w_r: jax.Array,
    B_w_gate: jax.Array,
    B_w_up: jax.Array,
    B_w_down: jax.Array,
):
    del B_x
    x = A_x.reshape(B, M)
    ckv = A_c_kv.reshape(B // 2, 2 * SK, DC)
    wq = A_w_q.reshape(M * H, D)
    wuk = A_w_uk.reshape(DC * H, D)
    wuv = A_w_uv.reshape(DC * H, D)
    wo = jnp.transpose(A_w_o, (0, 2, 1)).reshape(H * M, D)
    wd = B_w_down.T
    out = pl.pallas_call(
        _kernel,
        out_shape=jax.ShapeDtypeStruct((B, M), bf16),
        in_specs=[pl.BlockSpec(memory_space=pl.ANY)] * 10,
        out_specs=pl.BlockSpec(memory_space=pltpu.VMEM),
        scratch_shapes=[
            pltpu.VMEM((B, M), bf16),
            pltpu.VMEM((M,), bf16),
            pltpu.VMEM((M * H // 2, D), u32),
            pltpu.VMEM((DC * H // 2, D), u32),
            pltpu.VMEM((B // 2, 2 * SK, DC), bf16),
            pltpu.VMEM((DC * H // 2, D), u32),
            pltpu.VMEM((H * HR, D), u32),
            pltpu.VMEM((M, F), bf16),
            pltpu.VMEM((M, F), bf16),
            pltpu.VMEM((M, F), bf16),
            pltpu.VMEM((128, 128), f32),
            pltpu.VMEM((4, 128, 128), f32),
            pltpu.VMEM((SK // KC, H, KC), f32),
            pltpu.VMEM((4, 128, 128), f32),
            pltpu.VMEM((128, 2 * DC), f32),
            pltpu.VMEM((4 * H + 8, D), f32),
            pltpu.VMEM((8, F), f32),
            pltpu.SemaphoreType.DMA((N_SEMS,)),
        ],
        compiler_params=pltpu.CompilerParams(
            vmem_limit_bytes=100 * 1024 * 1024,
            disable_semaphore_checks=True,
            disable_bounds_checks=True,
        ),
    )(x, B_w_r, wq, wuk, ckv, wuv, wo, B_w_gate, B_w_up, wd)
    return out.reshape(B, 1, M)
```

```python
import jax
import jax.numpy as jnp
from jax import lax
from jax.experimental import pallas as pl
from jax.experimental.pallas import tpu as pltpu

B, H, SK, D, M, DC, F = 4, 32, 4096, 128, 576, 512, 4608
KC = 1024
NC = 512
HR = M // 2
MF = 512
G = 8
SHIFT = 6
LOOKAHEAD = 6
TAIL = tuple(range(3, H, 4))
N_SEMS = 2 + 11 + len(TAIL)
f32 = jnp.float32
bf16 = jnp.bfloat16
u32 = jnp.uint32


def _dot(a, b):
    return jnp.dot(a, b, preferred_element_type=f32)


def _dot_nt(a, b):
    return lax.dot_general(a, b, (((1,), (1,)), ((), ())), preferred_element_type=f32)


def _iota(shape, dim):
    return lax.broadcasted_iota(jnp.int32, shape, dim)


def _mul(k, c):
    return k * c if isinstance(k, int) else pl.multiple_of(k * c, c)


def _kernel(x_hbm, wr_hbm, wq_hbm, wuk_hbm, ckv_hbm, wuv_hbm, wo_hbm, wg_hbm, wu_hbm, wd_hbm,
            o_ref,
            x_v, wr_v, wq_v, wuk_v, ckv_v, wuv_v, wo_v, wg_v, wu_v, wd_v,
            q_s, qa_s, s_s, cc_s, lc_s, ctx_s, h_s, sems):
    def rows_unit(src, dst, row0, region_rows, r, step=None):
        def view(g, k):
            rows = pl.ds(row0 + g * region_rows + _mul(k, step or r), r)
            return src.at[rows], dst.at[rows]
        return view

    def ffn_unit(src, dst):
        def view(g, k):
            rows = pl.ds(g * (M // G) + _mul(k // 2, 8), 8)
            cols = pl.ds(_mul(k % 2, F // 2), F // 2)
            return src.at[rows, cols], dst.at[rows, cols]
        return view

    wo32 = wo_hbm.bitcast(u32)
    units = [('wq', 18, rows_unit(wq_hbm.bitcast(u32), wq_v, 0, 1152, 64)),
             ('wuk', 16, rows_unit(wuk_hbm.bitcast(u32), wuk_v, 0, 1024, 64)),
             ('ckv0', 32, rows_unit(ckv_hbm.at[0], ckv_v.at[0], 0, 1024, 32)),
             ('ckv1', 32, rows_unit(ckv_hbm.at[1], ckv_v.at[1], 0, 1024, 32)),
             ('wuv', 16, rows_unit(wuv_hbm.bitcast(u32), wuv_v, 0, 1024, 64)),
             ('wg', 18, ffn_unit(wg_hbm, wg_v)),
             ('wu', 18, ffn_unit(wu_hbm, wu_v)),
             ('wd', 18, ffn_unit(wd_hbm, wd_v)),
             ('woh', 2, rows_unit(wo32, wo_v, 2 * HR + MF // 2, 4 * HR, 32, HR)),
             ('wo0', 9, rows_unit(wo32, wo_v, 0, 4 * HR, 64)),
             ('wo1', 4, rows_unit(wo32, wo_v, 2 * HR, 4 * HR, 64))]
    tail = [(f'wt{h}', 1, rows_unit(wo32, wo_v, h * HR - 32, 32, 64)) for h in TAIL]
    sem_of = {u[0]: i + 2 for i, u in enumerate(units + tail)}
    assert len(sem_of) + 2 == N_SEMS
    rounds_a = [(u, k) for u in units for k in range(u[1])]
    rounds_b = rounds_a + [(u, 0) for u in tail]
    end = {u[0]: i + 1 for i, (u, _) in enumerate(rounds_a)}
    last = len(rounds_b) - SHIFT
    pos = [-SHIFT]

    def issue(ua, ka, ub, kb):
        for g in range(0, G, 2):
            for u, k, p in ((ub, kb, 1), (ua, ka, 0)):
                if u is not None:
                    src, dst = u[2](g + p, k)
                    pltpu.make_async_copy(src, dst, sems.at[sem_of[u[0]]]).start(priority=p)

    def take(n):
        lo, hi = pos[0], max(pos[0], min(pos[0] + n, last))
        pos[0] = hi
        out = []
        for rho in range(lo, hi):
            ua, ka = rounds_a[rho] if 0 <= rho < len(rounds_a) else (None, 0)
            ub, kb = rounds_b[rho + SHIFT]
            if out and out[-1][2] is ua and out[-1][4] is ub:
                out[-1][1] += 1
            else:
                out.append([rho - lo, 1, ua, ka, ub, kb])
        return out

    def issue_next(n):
        for _, cnt, ua, ka, ub, kb in take(n):
            if cnt == 1:
                issue(ua, ka, ub, kb)
            else:
                def body(i, _, ua=ua, ka=ka, ub=ub, kb=kb):
                    issue(ua, ka + i, ub, kb + i)
                    return 0
                lax.fori_loop(0, cnt, body, 0)

    def paced_loop(trips, n, step, body, init):
        assert (n - 1) * step < trips
        runs = take(n)

        def wrapped(i, carry):
            for lo, cnt, ua, ka, ub, kb in runs:
                cond = jnp.logical_and(i >= lo * step, i < (lo + cnt) * step)
                if step > 1:
                    cond = jnp.logical_and(cond, i % step == 0)

                @pl.when(cond)
                def _(lo=lo, cnt=cnt, ua=ua, ka=ka, ub=ub, kb=kb):
                    t = jnp.clip(i // step - lo, 0, cnt - 1) if cnt > 1 else 0
                    issue(ua, ka + t, ub, kb + t)
            return body(i, carry)
        return lax.fori_loop(0, trips, wrapped, init)

    def wait(name, *bufs):
        if name in end:
            issue_next(end[name] + LOOKAHEAD - pos[0])
        for buf in bufs:
            pltpu.make_async_copy(buf, buf, sems.at[sem_of[name]]).wait()

    c_x = pltpu.make_async_copy(x_hbm, x_v, sems.at[0])
    c_wr = pltpu.make_async_copy(wr_hbm, wr_v, sems.at[1])
    issue_next(1)
    c_x.start()
    c_wr.start()
    issue_next(SHIFT + 4)

    cc_s[...] = jnp.zeros(cc_s.shape, f32)
    ctx_s[pl.ds(4 * H, 8), :] = jnp.zeros((8, D), f32)
    c_x.wait()
    c_wr.wait()
    x = x_v[...].astype(f32)
    x = jnp.concatenate([x, x], axis=0)
    mu = jnp.mean(x, axis=-1, keepdims=True)
    xc = x - mu
    var = jnp.mean(xc * xc, axis=-1, keepdims=True)
    xn = (xc / jnp.sqrt(var + 1e-5)).astype(bf16).astype(f32)
    wr = wr_v[...].astype(f32).reshape(1, M)
    r = jnp.sum(xn * wr, axis=-1, keepdims=True)
    xn8 = xn.astype(bf16)
    E = (_iota((128, 256), 1) // 2 == _iota((128, 256), 0)).astype(f32).astype(bf16)
    ET = (_iota((256, 128), 0) // 2 == _iota((256, 128), 1)).astype(f32).astype(bf16)
    parts = [_dot(xn8[:, 128 * k:128 * (k + 1)], E) for k in range(4)]
    parts.append(_dot(xn8[:, 512:576], E[:64, :128]))
    lx = jnp.concatenate(parts, axis=1)
    lx = jnp.where(_iota((8, 2 * M), 0) // 4 == _iota((8, 2 * M), 1) % 2, lx, 0.0).astype(bf16)

    wait('wq', wq_v)

    def body_q(jj, _):
        ws = [pltpu.bitcast(wq_v[pl.ds(2 * jj + i, M, stride=16), :], bf16) for i in range(2)]
        res = _dot(lx, jnp.concatenate(ws, axis=1)) * (D ** -0.5)
        for i in range(2):
            q_s[pl.ds(pl.multiple_of(8 * (2 * jj + i), 8), 8), :] = res[:, 128 * i:128 * (i + 1)]
        return 0
    paced_loop(8, 8, 1, body_q, 0)
    issue_next(2)

    wait('wuk', wuk_v)
    pm = _iota((8, 2 * DC), 0) // 4 == _iota((8, 2 * DC), 1) % 2

    def body_qa(j, _):
        w = pltpu.bitcast(wuk_v[pl.ds(j, DC, stride=16), :], bf16)
        rows = pl.ds(pl.multiple_of(8 * j, 8), 8)
        lc_s[rows, :] = jnp.where(pm, _dot_nt(q_s[rows, :].astype(bf16), w), 0.0)
        return 0
    paced_loop(H // 2, 14, 1, body_qa, 0)
    rall = lc_s[...].astype(bf16)
    for k in range(4):
        qa_s[k] = _dot(rall[:, 256 * k:256 * (k + 1)], ET)

    for b in range(B):
        if b % 2 == 0:
            wait(f'ckv{b // 2}', ckv_v.at[b // 2])
        kv = ckv_v.at[b // 2, pl.ds((b % 2) * SK, SK)]
        qa = jnp.concatenate([qa_s[k, pl.ds(b, H, stride=4), :] for k in range(4)],
                             axis=1).astype(bf16)

        def body_s(i, mx, kv=kv, qa=qa):
            s = _dot_nt(qa, kv[pl.ds(pl.multiple_of(i * KC, KC), KC), :])
            s_s[i] = s
            for t in range(KC // 128):
                mx = jnp.maximum(mx, s[:, 128 * t:128 * (t + 1)])
            return mx
        mx = paced_loop(SK // KC, 4, 1, body_s, jnp.full((H, 128), -jnp.inf, f32))
        issue_next(1)
        mx = jnp.max(mx, axis=1, keepdims=True)

        def body_pv(i, carry, kv=kv, mx=mx):
            acc, l = carry
            p = jnp.exp(s_s[i] - mx)
            for t in range(KC // 128):
                l = l + p[:, 128 * t:128 * (t + 1)]
            kk = kv[pl.ds(pl.multiple_of(i * KC, KC), KC), :]
            return acc + _dot(p.astype(bf16), kk), l
        acc, l = paced_loop(SK // KC, 4, 1, body_pv,
                            (jnp.zeros((H, DC), f32), jnp.zeros((H, 128), f32)))
        issue_next(1)
        acc = acc / jnp.sum(l, axis=1, keepdims=True)
        for k in range(4):
            cc_s[k, pl.ds(b, H, stride=4), :] = acc[:, 128 * k:128 * (k + 1)]

    wait('wuv', wuv_v)
    pm2 = (_iota((128, 256), 0) // 4) % 2 == _iota((128, 256), 1) % 2
    for k in range(4):
        lc_s[:, 256 * k:256 * (k + 1)] = jnp.where(pm2, _dot(cc_s[k].astype(bf16), E), 0.0)

    def body_ctx(j, _):
        w = pltpu.bitcast(wuv_v[pl.ds(j, DC, stride=16), :], bf16)
        rows = pl.ds(pl.multiple_of(8 * j, 8), 8)
        ctx_s[rows, :] = _dot(lc_s[rows, :].astype(bf16), w)
        return 0
    issue_next(1)
    paced_loop(H // 2, 14, 1, body_ctx, 0)

    wait('wg', wg_v)

    def body_g(i, _):
        cols = pl.ds(pl.multiple_of(i * NC, NC), NC)
        h_s[:, cols] = _dot(xn8, wg_v[:, cols])
        return 0
    paced_loop(F // NC, 5, 2, body_g, 0)
    wait('wu', wu_v)

    def body_u(i, _):
        cols = pl.ds(pl.multiple_of(i * NC, NC), NC)
        g = h_s[:, cols]
        h_s[:, cols] = g * jax.nn.sigmoid(g) * _dot(xn8, wu_v[:, cols])
        return 0
    paced_loop(F // NC, 5, 2, body_u, 0)

    wait('wd', wd_v)

    def body_d(i, y):
        cols = pl.ds(pl.multiple_of(i * NC, NC), NC)
        return y + _dot_nt(h_s[:, cols].astype(bf16), wd_v[:, cols])
    y = paced_loop(F // NC, 8, 1, body_d, jnp.zeros((8, M), f32))
    t = xn + y * jax.nn.sigmoid(r)
    gate = t * jax.nn.sigmoid(t)

    def o_jobs(jobs, lo, hi):
        for h, r0, n in jobs:
            w = pltpu.bitcast(wo_v[pl.ds((h * M + r0) // 2, n // 2), :], bf16)
            res = _dot_nt(ctx_s[pl.ds(4 * h, 8), :].astype(bf16), w)
            if r0 == 0:
                lo = lo + res[:, :MF]
            if r0 + n == M:
                hi = hi + res[:, n - (M - MF):]
        return lo, hi

    issue_next(last - pos[0])
    late = [h for h in range(H) if h % 4 >= 2]
    wait('woh', *[wo_v.at[pl.ds(h * HR + MF // 2, HR - MF // 2)] for h in late])
    wait('wo0', *[wo_v.at[pl.ds(4 * g * HR, 2 * HR)] for g in range(G)])
    s_lo, s_hi = o_jobs([(h, 0, M) for h in range(H) if h % 4 < 2] + [(h, MF, M - MF) for h in late],
                        jnp.zeros((8, MF), f32), jnp.zeros((8, M - MF), f32))
    o_ref[:, MF:] = (x[:, MF:] + s_hi * gate[:, MF:]).astype(bf16)[:B]
    wait('wo1', *[wo_v.at[pl.ds(h * HR, MF // 2)] for h in range(2, H, 4)])
    s_lo, s_hi = o_jobs([(h, 0, MF) for h in range(2, H, 4)], s_lo, s_hi)
    for hs in (TAIL[:4], TAIL[4:6], TAIL[6:7]):
        for h in hs:
            wait(f'wt{h}', wo_v.at[pl.ds(h * HR, MF // 2)])
        s_lo, s_hi = o_jobs([(h, 0, MF) for h in hs], s_lo, s_hi)
    base = x[:, :MF] + s_lo * gate[:, :MF]
    c_last = ctx_s[pl.ds(4 * (H - 1), 8), :].astype(bf16)
    wait(f'wt{H - 1}', wo_v.at[pl.ds((H - 1) * HR, MF // 2)])
    w = pltpu.bitcast(wo_v[pl.ds((H - 1) * HR, MF // 2), :], bf16)
    o_ref[:, :MF] = (base + _dot_nt(c_last, w) * gate[:, :MF]).astype(bf16)[:B]


@jax.jit
def pallas_recurrent_scan__compressed_kv_cla__moe_arch_mod__decode_kernel(
    A_x: jax.Array,
    A_c_kv: jax.Array,
    A_w_q: jax.Array,
    A_w_uk: jax.Array,
    A_w_uv: jax.Array,
    A_w_o: jax.Array,
    B_x: jax.Array,
    B_w_r: jax.Array,
    B_w_gate: jax.Array,
    B_w_up: jax.Array,
    B_w_down: jax.Array,
):
    del B_x
    x = A_x.reshape(B, M)
    ckv = A_c_kv.reshape(B // 2, 2 * SK, DC)
    wq = A_w_q.reshape(M * H, D)
    wuk = A_w_uk.reshape(DC * H, D)
    wuv = A_w_uv.reshape(DC * H, D)
    wo = jnp.transpose(A_w_o, (0, 2, 1)).reshape(H * M, D)
    wd = B_w_down.T
    out = pl.pallas_call(
        _kernel,
        out_shape=jax.ShapeDtypeStruct((B, M), bf16),
        in_specs=[pl.BlockSpec(memory_space=pl.ANY)] * 10,
        out_specs=pl.BlockSpec(memory_space=pltpu.VMEM),
        scratch_shapes=[
            pltpu.VMEM((B, M), bf16),
            pltpu.VMEM((M,), bf16),
            pltpu.VMEM((M * H // 2, D), u32),
            pltpu.VMEM((DC * H // 2, D), u32),
            pltpu.VMEM((B // 2, 2 * SK, DC), bf16),
            pltpu.VMEM((DC * H // 2, D), u32),
            pltpu.VMEM((H * HR, D), u32),
            pltpu.VMEM((M, F), bf16),
            pltpu.VMEM((M, F), bf16),
            pltpu.VMEM((M, F), bf16),
            pltpu.VMEM((128, 128), f32),
            pltpu.VMEM((4, 128, 128), f32),
            pltpu.VMEM((SK // KC, H, KC), f32),
            pltpu.VMEM((4, 128, 128), f32),
            pltpu.VMEM((128, 2 * DC), f32),
            pltpu.VMEM((4 * H + 8, D), f32),
            pltpu.VMEM((8, F), f32),
            pltpu.SemaphoreType.DMA((N_SEMS,)),
        ],
        compiler_params=pltpu.CompilerParams(
            vmem_limit_bytes=100 * 1024 * 1024,
            disable_semaphore_checks=True,
            disable_bounds_checks=True,
        ),
    )(x, B_w_r, wq, wuk, ckv, wuv, wo, B_w_gate, B_w_up, wd)
    return out.reshape(B, 1, M)
```
